```python
import os as _os
_os.environ.setdefault("JAX_PLATFORMS", "cpu")
import jax
import jax.numpy as jnp

def _softmax(x, axis=-1):
    return jax.nn.softmax(x, axis=axis)
def _gelu(x):
    return jax.nn.gelu(x, approximate=True)
def _silu(x):
    return jax.nn.silu(x)
def _sigmoid(x):
    return jax.nn.sigmoid(x)
def _layernorm(x, axis=-1, eps=1e-5):
    m = jnp.mean(x, axis=axis, keepdims=True)
    v = jnp.var(x, axis=axis, keepdims=True)
    return (x - m) / jnp.sqrt(v + eps)
def _scatter_add(tgt, idx, src, axis=0):
    return tgt.at[idx].add(src)
def _segment_sum(src, seg, n):
    return jax.ops.segment_sum(src, seg, n)
class _Rng:
    def __init__(self, key):
        self._k = key
    def _next(self):
        self._k, sub = jax.random.split(self._k)
        return sub
    def normal(self, shape):
        return jax.random.normal(self._next(), shape, dtype=jnp.bfloat16)
    def randint(self, lo, hi, shape):
        return jax.random.randint(self._next(), shape, lo, hi, dtype=jnp.int32)
    def uniform(self, shape, lo=0.0, hi=1.0):
        return jax.random.uniform(self._next(), shape, jnp.bfloat16, lo, hi)
    def permutation(self, n):
        return jax.random.permutation(self._next(), n)


kernel_name = 'parallel_sum__ssm_conv_h3__dense_activation_silu__prompt'

def setup_inputs():
    _rng = _Rng(jax.random.key(int.from_bytes(__import__("os").urandom(4), "little")))
    _w = (lambda a: (lambda t: t.astype(jnp.bfloat16) if jnp.issubdtype(t.dtype, jnp.floating) else t)(jnp.asarray(a)))
    def _A_setup():
        B, S, D = 1, 2048, 448
        ks = 4
        return {
            "q": _w((lambda *s: _rng.normal(s) * 0.05)(B, S, D)),
            "k": _w((lambda *s: _rng.normal(s) * 0.2)(B, S, D)),
            "v": _w((lambda *s: _rng.normal(s) * 0.2)(B, S, D)),
            "shift_k": _w((lambda *s: _rng.normal(s) * 0.2)(D, ks) * 0.5),
            "ssm_k": _w((lambda *s: _rng.normal(s) * 0.2)(D, S) * (1.0 / S ** 0.5)),
            "ssm_D": _w((lambda *s: _rng.normal(s) * 0.2)(D)),
        }
    _A_in = _A_setup()

    def _B_setup():
        B, S, D, F = 1, 2048, 448, 1792
        return {
            "x": _w((lambda *s: _rng.normal(s) * 0.05)(B, S, D)),
            "w1": _w((lambda *s: _rng.normal(s) * 0.05)(D, F) * (D ** -0.5)),
            "w2": _w((lambda *s: _rng.normal(s) * 0.05)(F, D) * (F ** -0.5)),
        }
    _B_in = _B_setup()

    return {
        "A_q": _A_in["q"],
        "A_k": _A_in["k"],
        "A_v": _A_in["v"],
        "A_shift_k": _A_in["shift_k"],
        "A_ssm_k": _A_in["ssm_k"],
        "A_ssm_D": _A_in["ssm_D"],
        "B_x": _B_in["x"],
        "B_w1": _B_in["w1"],
        "B_w2": _B_in["w2"],
    }

def reference(A_q, A_k, A_v, A_shift_k, A_ssm_k, A_ssm_D, B_x, B_w1, B_w2):
    def _A_ref(q, k, v, shift_k, ssm_k, ssm_D):
        B, S, D = q.shape
        ks = shift_k.shape[-1]
        k_pad = jnp.pad(k, ((0, 0), (ks - 1, 0), (0, 0)))
        k_shift = jnp.zeros_like(k)
        for t in range(ks):
            k_shift = k_shift + k_pad[:, t:t + S, :] * shift_k[:, ks - 1 - t][None, None, :]
        kv = k_shift * v
        L = 2 * S
        kv_pad = jnp.pad(kv, ((0, 0), (0, S), (0, 0)))
        kf_pad = jnp.pad(ssm_k, ((0, 0), (0, S)))
        kv_f = (lambda x, axes=(-2,-1): jnp.fft.rfft2(x.astype(jnp.float32), axes=axes))(kv_pad[:, None, :, :], axes=(1, 2))
        kf_f = (lambda x, axes=(-2,-1): jnp.fft.rfft2(x.astype(jnp.float32), axes=axes))(kf_pad[:, None, :], axes=(1, 2))
        kf_f = (lambda x, *d: x.transpose(*d))(kf_f, 1, 2, 0)
        y_f = kv_f * kf_f[None, :, :, :]
        y = (lambda x, s, axes=(-2,-1): jnp.fft.irfft2(x, s=s, axes=axes).astype(jnp.bfloat16))(y_f, (1, L), axes=(1, 2))[:, 0, :S, :]
        y = y + kv * ssm_D[None, None, :]
        return q * y

    def _B_ref(x, w1, w2):
        h = jnp.einsum("bsd,df->bsf", x, w1)
        h = _silu(h)
        out = jnp.einsum("bsf,fd->bsd", h, w2)
        return out

    x = A_q
    xn = _layernorm(x, axis=-1)
    return x + _A_ref(xn, A_k, A_v, A_shift_k, A_ssm_k, A_ssm_D) + _B_ref(xn, B_w1, B_w2)
```

```python
import jax
import jax.numpy as jnp
import numpy as np
from jax import lax
import jax.experimental.pallas as pl
import jax.experimental.pallas.tpu as pltpu

S, D, F = 2048, 448, 1792
C = 128
A = S // C
BF = jnp.bfloat16
F32 = jnp.float32
U32 = jnp.uint32
PAD = 16


def _dft_consts():
    n = np.arange(C, dtype=np.float64)[:, None]
    f = np.arange(C, dtype=np.float64)[None, :]
    ang = 2.0 * np.pi * n * (f + 0.5) / (2 * C)
    fw = np.concatenate([np.cos(ang), -np.sin(ang)], axis=1)
    fi = np.concatenate([np.cos(ang.T), -np.sin(ang.T)], axis=0) * (2.0 * 2.0 / (2 * C))
    return fw.astype(np.float32), fi.astype(np.float32)


_FW, _FI = _dft_consts()


def tree_sum(xs):
    xs = list(xs)
    while len(xs) > 1:
        nxt = [xs[i] + xs[i + 1] for i in range(0, len(xs) - 1, 2)]
        if len(xs) % 2:
            nxt.append(xs[-1])
        xs = nxt
    return xs[0]


def make(TS=256, c1=(512, 512, 512, 256), c2=(512, 512, 512, 256), nper=(1, 1, 1, 0, 2, 1, 0, 2), start=0,
         flags=None, waitall=True, opq=True, gx=True, gln=True, invh=2, tok=True, ntiles=None, xlead=2, finper=2,
         lnpos=0, waits=None, flead=None, ilag=None, finv=False, anchor=None, fine=False, phase=False, width=0, wdesc=False, pl2=2, odma=None, lo=0.03, hi=0.97, pdesc=False, split=False, dbg=False):
    NT = ntiles or S // TS
    N1, N2 = len(c1), len(c2)
    o1 = [sum(c1[:i]) for i in range(N1)]
    o2 = [sum(c2[:i]) for i in range(N2)]
    NV = 7 * A
    O_C, O_P, O_Q, O_S, O_XR, O_XI, O_K1 = (i * A for i in range(7))
    NSL = 4
    NXL = 64
    slots = []
    for t in range(NT):
        slots += [("f1", t, c) for c in range(N1)] + [("f2", t, c) for c in range(N2)]
    cnt = [nper[i % (N1 + N2)] if i >= start else 0 for i in range(len(slots))]
    NG = D // 8
    if ntiles is not None:
        NG = min(NG, sum(cnt[:-(N1 + N2)]))
    RB = 64
    NB = (NG * 8 + RB - 1) // RB

    def body(q_hbm, k_hbm, v_hbm, sh_hbm, sk_hbm, sd_hbm, w1_hbm, w2_hbm, fw_hbm, fi_hbm, o_hbm,
             q_v, kv_v, sk_v, w1_v, sh_v, sd_v, fw_v, fi_v,
             w1t_p, w2_v, w2_p, hh, wb0, wb1, tab_v, st_v, pw_v, k1_v, xl_v, y_v, b_v, o_v, sem, osem, zsem):
        wbs = [wb0, wb1]
        cps = {}
        nsem = [0]
        def start_dma(name, src, dst):
            c = pltpu.make_async_copy(src, dst, sem.at[nsem[0]]); nsem[0] += 1
            c.start(); cps[name] = c
        def wait(*names):
            for name in names:
                c = cps.pop(name, None)
                if c is not None:
                    if dbg: print("wait", name)
                    c.wait()
        def dma_q(t):
            sl = slice(t * TS, (t + 1) * TS)
            start_dma(("q", t), q_hbm.at[:, sl], q_v.at[0:D, sl])
        def dma_w1(c):
            sl = slice(c * (F // 2), (c + 1) * (F // 2))
            start_dma(("w1", c), w1_hbm.at[:, sl], w1_v.at[:, sl])
        def dma_w2(c):
            sl = slice(c * (F // 2), (c + 1) * (F // 2))
            start_dma(("w2", c), w2_hbm.at[:, sl], w2_v.at[:, sl])
        def dma_conv(b):
            rs = slice(b * RB, (b + 1) * RB)
            start_dma(("sk", b), sk_hbm.at[rs, :], sk_v.at[rs, :])
            start_dma(("k", b), k_hbm.at[rs, :], kv_v.at[rs, :])
            start_dma(("v", b), v_hbm.at[rs, :], kv_v.at[slice(D + b * RB, D + (b + 1) * RB), :])

        if opq:
            z0 = pl.semaphore_read(zsem.at[0])
            z16 = pl.multiple_of(z0 * 16, 16)
        else:
            z0 = z16 = 0

        lastbf = [None]
        def gate(ref, row):
            if opq and lastbf[0] is not None:
                ref[pl.ds(row + z16, 16), 0:C] = lastbf[0]

        def tabs():
            wait("sh", "sd")
            sh = sh_v[...].astype(F32)
            for j in range(4):
                tab_v[j] = jnp.broadcast_to(sh[j:j + 1], (128, D)).T
            sd = sd_v[...].astype(F32).reshape(1, D)
            tab_v[4] = jnp.broadcast_to(sd, (128, D)).T

        xnv = {}
        def ln_tile(t):
            wait(("q", t))
            sl = slice(t * TS, (t + 1) * TS)
            x = q_v[0:D, sl].astype(F32)
            xs = [x[i * 8:(i + 1) * 8] for i in range(D // 8)]
            m = jnp.sum(tree_sum(xs), axis=0, keepdims=True) * (1.0 / D)
            xc = [xi - m for xi in xs]
            var = jnp.sum(tree_sum([c * c for c in xc]), axis=0, keepdims=True) * (1.0 / D)
            r = 0.5 * lax.rsqrt(var + 1e-5)
            st_v[0:1, sl] = m
            st_v[1:2, sl] = r
            xf_ = jnp.concatenate(xc, axis=0) * r
            xnv[t] = [xf_[:, n * C:(n + 1) * C].astype(BF) for n in range(2)] if split else xf_.astype(BF)

        def w1_tr(c):
            wait(("w1", c))
            for j in range(c * 7, (c + 1) * 7):
                w1t_p[j * 64:(j + 1) * 64, :] = pltpu.bitcast(w1_v[:, j * 128:(j + 1) * 128].T, U32)

        def w2_pack(c):
            wait(("w2", c))
            sl = slice(c * (F // 2), (c + 1) * (F // 2))
            w2_p[:, sl] = pltpu.bitcast(w2_v[:, sl], U32)

        pend = []
        nanc = [0]
        def mkanchor(buf):
            i = nanc[0] % 8; nanc[0] += 1
            if isinstance(buf, str):
                pw_v[NSL * NV + 8 + i] = jnp.zeros((8, C), F32)
                return pltpu.bitcast(pw_v[NSL * NV + 8 + i], U32)
            else:
                buf[2, i * 16:i * 16 + 16, :] = jnp.zeros((16, C), BF)
                return pltpu.bitcast(buf[2, i * 16:i * 16 + 16, :].astype(F32)[0:8], U32)
        def anchored(ref, r0, r1, anc):
            x = ref[r0:r1, :]
            if not anc: return x
            parts = []; p = 0
            mer = {}
            for (r, z) in anc: mer[r] = (mer[r] | z) if r in mer else z
            for (r, z) in sorted(mer.items(), key=lambda t: t[0]):
                if r > p: parts.append(x[p:r])
                blk = x[r:r + 8]
                n = blk.shape[1]
                parts.append(blk | jnp.concatenate([z] * (-(-n // C)), axis=1)[:, :n])
                p = r + 8
            if p < r1 - r0: parts.append(x[p:])
            return jnp.concatenate(parts, axis=0)

        def take(nrows):
            out = [[], []]
            for a, z in pend:
                x = min(a, 0.9999) * 2
                rnd = int(x); out[rnd].append((int((x - rnd) * nrows) // 8 * 8, z))
            pend.clear()
            return out

        def f1(t, c):
            if split:
                anc = take(c1[c] // 2)
                u = jnp.concatenate([jnp.dot(pltpu.bitcast(anchored(w1t_p, o1[c] // 2, (o1[c] + c1[c]) // 2, anc[n]), BF),
                                             xnv[t][n], preferred_element_type=F32) for n in range(2)], axis=1)
            else:
                anc = [(int(a * c1[c] / 2) // 8 * 8, z) for a, z in pend]; pend.clear()
                lhs = pltpu.bitcast(anchored(w1t_p, o1[c] // 2, (o1[c] + c1[c]) // 2, anc), BF)
                u = jnp.dot(lhs, xnv[t], preferred_element_type=F32)
            hf = u + u * jnp.tanh(u)
            for j in range(N2):
                lo = max(o1[c], o2[j]); hi = min(o1[c] + c1[c], o2[j] + c2[j])
                if lo < hi:
                    hh[j][pl.ds(z16 + lo - o2[j], hi - lo), :] = hf[lo - o1[c]:hi - o1[c]].astype(BF)
            lastbf[0] = u[c1[c] - 16:c1[c], TS - C:TS].astype(BF)

        facc = {}
        def f2(t, c):
            sl = slice(o2[c], o2[c] + c2[c])
            if split:
                anc = take(D // 2)
                o = jnp.concatenate([jnp.dot(pltpu.bitcast(anchored(w2_p.at[:, sl], 0, D // 2, anc[n]), BF),
                                             hh[c][:, n * C:(n + 1) * C], preferred_element_type=F32) for n in range(2)], axis=1)
            else:
                anc = [(int(a * D / 2) // 8 * 8, z) for a, z in pend]; pend.clear()
                o = jnp.dot(pltpu.bitcast(anchored(w2_p.at[:, sl], 0, D // 2, anc), BF), hh[c][...], preferred_element_type=F32)
            facc[t] = o if c == 0 else facc[t] + o
            lastbf[0] = o[D - 16:D, TS - C:TS].astype(BF)

        def park(t):
            b_v[:, t * TS:(t + 1) * TS] = facc.pop(t)

        lane8 = lax.broadcasted_iota(jnp.int32, (8, C), 1)
        sg = (1 - 2 * (lane8 & 1)).astype(F32)

        def kfwd(g):
            wait(("sk", g * 8 // RB), "fw")
            kl = jnp.concatenate([sk_v[g * 8:g * 8 + 8, a * C:(a + 1) * C] for a in range(A)], axis=0)
            kh = jnp.dot(kl, fw_v[...], preferred_element_type=F32)
            base = (g % NSL) * NV
            kr = [kh[a * 8:a * 8 + 8, 0:C] for a in range(A)]
            ki = [kh[a * 8:a * 8 + 8, C:2 * C] for a in range(A)]
            kr[0] = kr[0] + tab_v[4, g * 8:g * 8 + 8, :]
            for a in range(A):
                cr = kr[a] if a == 0 else kr[a] - sg * ki[a - 1]
                ci = ki[a] if a == 0 else ki[a] + sg * kr[a - 1]
                pw_v[z0 + base + O_C + a] = cr
                pw_v[z0 + base + O_P + a] = ci - cr
                pw_v[z0 + base + O_Q + a] = -ci - cr

        xlv = {}
        def xpre(g):
            wait(("k", g * 8 // RB), ("v", g * 8 // RB))
            rs = slice(g * 8, g * 8 + 8)
            kf_ = kv_v[rs, :].astype(F32)
            vf = kv_v[D + g * 8:D + g * 8 + 8, :].astype(F32)
            lane = lax.broadcasted_iota(jnp.int32, (8, C), 1)
            tiles = []
            rolled = [kf_] + [pltpu.roll(kf_, j, 1) for j in range(1, 4)]
            w = [tab_v[j, rs, :] for j in range(4)]
            for a in range(A):
                sl = slice(a * C, (a + 1) * C)
                acc = kf_[:, sl] * w[0]
                for j in range(1, 4):
                    r = rolled[j][:, sl]
                    if a == 0:
                        r = jnp.where(lane >= j, r, 0.0)
                    acc = acc + r * w[j]
                tiles.append(acc * vf[:, sl])
            if phase:
                xl_v[g % NXL, pl.ds(z16, A * 8), :] = jnp.concatenate(tiles, axis=0).astype(BF)
            else:
                xlv[g] = jnp.concatenate(tiles, axis=0).astype(BF)

        def xfwd(g):
            wait("fw")
            xh = jnp.dot(xl_v[g % NXL] if phase else xlv.pop(g), fw_v[...], preferred_element_type=F32)
            base = (g % NSL) * NV
            for a in range(A):
                xr = xh[a * 8:a * 8 + 8, 0:C]
                xi = xh[a * 8:a * 8 + 8, C:2 * C]
                pw_v[z0 + base + O_XR + a] = xr
                pw_v[z0 + base + O_XI + a] = xi
                pw_v[z0 + base + O_S + a] = xr + xi

        def conv(base, oc, ox, init):
            cs = [pw_v[base + oc + a] for a in range(A)]
            xs = [pw_v[base + ox + a] for a in range(A)]
            out = []
            for a in range(A):
                acc = cs[0] * xs[a]
                if init is not None:
                    acc = acc + init(a)
                for dl in range(1, a + 1):
                    acc = acc + cs[dl] * xs[a - dl]
                out.append(acc)
            return out

        def pw_fine(g, p0, p1):
            base = (g % NSL) * NV
            kb = (g % 2) * 48
            def chain(oc, ox, a, init):
                acc = pw_v[base + oc] * pw_v[base + ox + a]
                if init is not None: acc = acc + init
                for dl in range(1, a + 1):
                    acc = acc + pw_v[base + oc + dl] * pw_v[base + ox + a - dl]
                return acc
            def anc(pos):
                i = nanc[0] % 16; nanc[0] += 1
                k1_v[kb + 24 + i] = jnp.zeros((8, C), F32)
                pend.append((p0 + (p1 - p0) * pos, pltpu.bitcast(k1_v[kb + 24 + i], U32)))
            prs = list(range(0, A, 2))
            if pdesc: prs = prs[::-1]
            tot = 3 * 136; done = 0
            for a in prs:
                for b in (a, a + 1):
                    k1_v[z0 + kb + b] = chain(O_C, O_S, b, None)
                done += 2 * a + 3; anc(done / tot)
            for half, (oc, ox) in ((1, (O_P, O_XR)), (0, (O_Q, O_XI))):
                for a in prs:
                    r = [chain(oc, ox, b, k1_v[kb + b]) for b in (a, a + 1)]
                    wbs[g % 2][half, pl.ds(z16 + a * 8, 16), :] = jnp.concatenate(r, axis=0).astype(BF)
                    k1_v[z0 + kb + 16] = r[0] + r[1]
                    done += 2 * a + 3; anc(done / tot)

        def pw_chain(g):
            base = (g % NSL) * NV
            TOK = NSL * NV
            def chains(oc, ox, aa, init):
                top = max(aa)
                cs = [pw_v[base + oc + i] for i in range(top + 1)]
                xs = [pw_v[base + ox + i] for i in range(top + 1)]
                out = []
                for a in aa:
                    acc = cs[0] * xs[a]
                    if init: acc = acc + pw_v[base + O_K1 + a]
                    for dl in range(1, a + 1):
                        acc = acc + cs[dl] * xs[a - dl]
                    out.append(acc)
                return out
            steps = [list(range(a, a + width)) for a in range(0, A, width)]
            if wdesc: steps = steps[::-1]
            for aa in steps:
                for a, r in zip(aa, chains(O_C, O_S, aa, False)):
                    pw_v[z0 + base + O_K1 + a] = r
            for half, (oc, ox) in ((1, (O_P, O_XR)), (0, (O_Q, O_XI))):
                for aa in steps:
                    r = chains(oc, ox, aa, True)
                    wbs[g % 2][half, pl.ds(z16 + aa[0] * 8, 8 * width), :] = jnp.concatenate(r, axis=0).astype(BF)
                    for i in range(0, width, 2):
                        pw_v[z0 + TOK + i // 2] = r[i] + r[i + 1] if tok == 2 else r[i + 1]
            if anchor is not None:
                pend.append((anchor, mkanchor("pw")))

        def pw(g):
            base = (g % NSL) * NV
            TOK = NSL * NV
            k1 = conv(base, O_C, O_S, None)
            for a in range(A):
                pw_v[z0 + base + O_K1 + a] = k1[a]
            ld = lambda a: pw_v[base + O_K1 + a]
            wim = conv(base, O_P, O_XR, ld)
            wbs[g % 2][1, pl.ds(z16, A * 8), :] = jnp.concatenate(wim, axis=0).astype(BF)
            if tok:
                pw_v[z0 + TOK] = wim[A - 1]
            wre = conv(base, O_Q, O_XI, ld)
            wbs[g % 2][0, pl.ds(z16, A * 8), :] = jnp.concatenate(wre, axis=0).astype(BF)
            if tok:
                pw_v[z0 + TOK + 1] = wre[A - 1]
            if anchor is not None:
                pend.append((anchor, mkanchor("pw")))

        def inv(g):
            wait("fi")
            n = A // invh
            for hh in range(invh):
                rows = slice(hh * n * 8, (hh + 1) * n * 8)
                w = jnp.concatenate([wbs[g % 2][0, rows, :], wbs[g % 2][1, rows, :]], axis=1)
                y = jnp.dot(w, fi_v[...], preferred_element_type=F32)
                for a in range(n):
                    y_v[g * 8:g * 8 + 8, (hh * n + a) * C:(hh * n + a + 1) * C] = y[a * 8:a * 8 + 8, :]

        ocs = []; fdone = []; ostart = [0]
        def fin(t, parked=True):
            sl = slice(t * TS, (t + 1) * TS)
            B = b_v[:, sl] if parked else facc.pop(t)
            x = q_v[0:D, sl].astype(F32)
            xn = (x - st_v[0:1, sl]) * st_v[1:2, sl]
            o_v[:, sl] = (x + xn * y_v[:, sl] + B).astype(BF)
            fdone.append(t)
            if odma is None or t in odma:
                t0 = ostart[0]; ostart[0] = t + 1
                assert sorted(fdone) == list(range(t + 1)) or odma is None
                s2 = slice(t * TS, (t + 1) * TS) if odma is None else slice(t0 * TS, (t + 1) * TS)
                c = pltpu.make_async_copy(o_v.at[:, s2], o_hbm.at[:, s2], osem.at[t]); c.start()
                ocs.append(c)

        start_dma("sh", sh_hbm, sh_v); start_dma("sd", sd_hbm, sd_v)
        start_dma("fw", fw_hbm, fw_v); start_dma("fi", fi_hbm, fi_v)
        started = set()
        def kick(names):
            for nm in names:
                if nm == "all":
                    kick([("w1", 0), ("w1", 1), ("w2", 0), ("w2", 1)] + [("q", t) for t in range(NT)] + [("conv", b) for b in range(NB)])
                elif nm not in started:
                    started.add(nm)
                    {"q": dma_q, "w1": dma_w1, "w2": dma_w2, "conv": dma_conv}[nm[0]](nm[1])
        if waits is None: kick([("q", 0), ("w1", 0), ("w1", 1), ("conv", 0), "all"])
        else: kick(waits[-2])
        if waitall:
            wait(*list(cps.keys()))

        def barrier(names):
            for nm in names:
                if nm == "all": wait(*list(cps.keys()))
                elif isinstance(nm, tuple) and nm[0] == "conv": wait(("sk", nm[1]), ("k", nm[1]), ("v", nm[1]))
                else: wait(nm)
        setup = {"w1a": lambda: w1_tr(0), "w1b": lambda: w1_tr(1), "w2a": lambda: w2_pack(0), "w2b": lambda: w2_pack(1), "tabs": tabs}
        def run_setup(si):
            if waits is None:
                if si == -1:
                    for k_ in ("w1a", "w1b", "w2a", "w2b", "tabs"): setup[k_]()
                return
            if si in waits:
                barrier(waits[si][0])
                kick(waits[si][2])
                for k_ in waits[si][1]: setup[k_]()
        if waits is not None and -1 in waits: barrier(waits[-1][0]); kick(waits[-1][2])
        ln_tile(0)
        run_setup(-1)

        gl = []
        g = 0
        for si in range(len(slots)):
            n = min(cnt[si], NG - g)
            gl.append(list(range(g, g + n))); g += n
        assert g == NG, (g, NG)
        nxt = lambda si: next((gl[j] for j in range(si + 1, len(slots)) if gl[j]), [])
        order = [x for l in gl for x in l]
        last_inv_slot = max(si + (ilag[si % (N1 + N2)] if ilag else 0) for si in range(len(slots)) if gl[si])
        fins = []
        done_fwd = set(); done_pre = set()
        def do_pre(gs):
            for x in gs:
                if x < NG and x not in done_pre:
                    if gx: gate(kv_v, 2 * D)
                    xpre(x); done_pre.add(x)
        def do_fwd(gs):
            for x in sorted(gs):
                if x < NG and x not in done_fwd:
                    do_pre([x])
                    kfwd(x); xfwd(x); done_fwd.add(x)
        for si, (kind, t, c) in enumerate(slots):
            run_setup(si)
            for n, g in enumerate(gl[si] if not phase else []):
                if fine:
                    m = len(gl[si])
                    pw_fine(g, lo + (hi - lo) * n / m, lo + (hi - lo) * (n + 1) / m)
                elif width:
                    pw_chain(g)
                else:
                    pw(g)
            if kind == "f1":
                f1(t, c)
            else:
                f2(t, c)
                if c == N2 - 1:
                    if si < last_inv_slot: park(t); fins.append(t)
                    else: fins.append(-t - 1)
            if (kind, c) == (("f1", lnpos) if lnpos < N1 else ("f2", lnpos - N1)) and t + 1 < NT:
                if gln: gate(q_v, D)
                ln_tile(t + 1)
            fw_now = []
            for j in range(si + 1, min(len(slots), si + 4)):
                ld = 1 + (flead[j % (N1 + N2)] if flead else 0)
                if j - ld == si: fw_now += gl[j]
            iv_now = []
            for j in range(max(0, si - 2), si + 1):
                lg = (ilag[j % (N1 + N2)] if ilag else 0)
                if j + lg == si or (si == len(slots) - 1 and j + lg > si): iv_now += gl[j]
            if phase:
                gs = gl[si]
                for n, g in enumerate(gs):
                    pw(g)
                    if finv:
                        inv(g)
                        if n + pl2 < len(gs): do_fwd([gs[n + pl2]])
                    else:
                        if n + pl2 < len(gs): do_fwd([gs[n + pl2]])
                        inv(g)
                if si + 1 < len(slots): do_fwd(gl[si + 1][:pl2])
            elif finv:
                for g in iv_now: inv(g)
                do_fwd(fw_now)
            else:
                do_fwd(fw_now)
                for g in iv_now: inv(g)
            if phase:
                nx = next((j for j in range(si + 1, len(slots)) if gl[j]), None)
                if nx is not None:
                    todo = [g for g in gl[nx] if g not in done_pre]
                    left = nx - si
                    k = -(-len(todo) // left)
                    do_pre(todo[:k])
            else:
              for j in range(si + 2, min(len(slots), si + 5)):
                ld = 1 + (flead[j % (N1 + N2)] if flead else 0)
                if j - ld == si + 1: do_pre(gl[j])
            if si >= last_inv_slot:
                nrem = len(slots) - 1 - si
                k = len(fins) if nrem == 0 else min(len(fins), max(finper, -(-len(fins) // nrem)))
                for _ in range(k):
                    x = fins.pop(0)
                    if x >= 0: fin(x)
                    else: fin(-x - 1, parked=False)
        assert not fins, fins
        for c in ocs:
            c.wait()
        assert not cps, cps.keys()

    NSEM = 4 + NT + 4 + 3 * NB

    def run(A_q, A_k, A_v, A_shift_k, A_ssm_k, A_ssm_D, B_x, B_w1, B_w2):
        qT = A_q[0].T; kT = A_k[0].T; vT = A_v[0].T
        anyspec = pl.BlockSpec(memory_space=pl.ANY)
        o = pl.pallas_call(
            body,
            out_shape=jax.ShapeDtypeStruct((D, S), BF),
            in_specs=[anyspec] * 10,
            out_specs=anyspec,
            scratch_shapes=[
                pltpu.VMEM((D + PAD, S), BF), pltpu.VMEM((2 * D + PAD, S), BF), pltpu.VMEM((D, S), BF),
                pltpu.VMEM((D, F), BF),
                pltpu.VMEM((4, D), BF), pltpu.VMEM((D,), BF), pltpu.VMEM((C, 2 * C), BF), pltpu.VMEM((2 * C, C), BF),
                pltpu.VMEM((F // 2, D), U32), pltpu.VMEM((D, F), BF), pltpu.VMEM((D // 2, F), U32),
                [pltpu.VMEM((n, TS), BF) for n in c2],
                pltpu.VMEM((3, A * 8, C), BF), pltpu.VMEM((3, A * 8, C), BF),
                pltpu.VMEM((5, D, 128), F32), pltpu.VMEM((8, S), F32),
                pltpu.VMEM((NSL * NV + 16, 8, C), F32), pltpu.VMEM((96, 8, C), F32), pltpu.VMEM((NXL, A * 8, C), BF),
                pltpu.VMEM((D, S), F32), pltpu.VMEM((D, S), F32), pltpu.VMEM((D, S), BF),
                pltpu.SemaphoreType.DMA((NSEM,)), pltpu.SemaphoreType.DMA((NT,)), pltpu.SemaphoreType.REGULAR((2,)),
            ],
            compiler_params=pltpu.CompilerParams(vmem_limit_bytes=100 * 1024 * 1024, flags=flags),
            name="h3ffn",
        )(qT, kT, vT, A_shift_k.T, A_ssm_k, A_ssm_D, B_w1, B_w2.T, jnp.asarray(_FW, BF), jnp.asarray(_FI, BF))
        return o.T[None]
    return run


@jax.jit
def pallas_parallel_sum__ssm_conv_h3__dense_activation_silu__prompt_kernel(
    A_q, A_k, A_v, A_shift_k, A_ssm_k, A_ssm_D, B_x, B_w1, B_w2,
):
    return make(c1=(448,448,448,448),c2=(512,512,768),lnpos=4,waitall=False,nper=(1,1,2,1,1,1,2),start=5,width=4,tok=2,finv=True,waits={-2:[('q',0),('w1',0)], -1:(['sh','sd','fw','fi',('q',0),('w1',0)],['w1a'],[('w1',1),('w2',0)]), 1:([('w1',1),('w2',0)],['w1b','w2a','tabs'],[('w2',1),('q',1),('conv',0)]), 3:([('w2',1),('q',1),('conv',0)],['w2b'],[('conv',1),('q',2),('conv',2),('q',3)]), 7:([('conv',1),('q',2),('conv',2),('q',3)],[],['all']), 14:(['all'],[],[])},odma=(2,4,5,6,7))(A_q, A_k, A_v, A_shift_k, A_ssm_k, A_ssm_D, B_x, B_w1, B_w2)
```
